```python
import os as _os
_os.environ.setdefault("JAX_PLATFORMS", "cpu")
import jax
import jax.numpy as jnp

def _softmax(x, axis=-1):
    return jax.nn.softmax(x, axis=axis)
def _gelu(x):
    return jax.nn.gelu(x, approximate=True)
def _silu(x):
    return jax.nn.silu(x)
def _sigmoid(x):
    return jax.nn.sigmoid(x)
def _layernorm(x, axis=-1, eps=1e-5):
    m = jnp.mean(x, axis=axis, keepdims=True)
    v = jnp.var(x, axis=axis, keepdims=True)
    return (x - m) / jnp.sqrt(v + eps)
def _scatter_add(tgt, idx, src, axis=0):
    return tgt.at[idx].add(src)
def _segment_sum(src, seg, n):
    return jax.ops.segment_sum(src, seg, n)
class _Rng:
    def __init__(self, key):
        self._k = key
    def _next(self):
        self._k, sub = jax.random.split(self._k)
        return sub
    def normal(self, shape):
        return jax.random.normal(self._next(), shape, dtype=jnp.bfloat16)
    def randint(self, lo, hi, shape):
        return jax.random.randint(self._next(), shape, lo, hi, dtype=jnp.int32)
    def uniform(self, shape, lo=0.0, hi=1.0):
        return jax.random.uniform(self._next(), shape, jnp.bfloat16, lo, hi)
    def permutation(self, n):
        return jax.random.permutation(self._next(), n)


kernel_name = 'standalone__cross_network_dcn_v2__recsys'

def setup_inputs():
    _rng = _Rng(jax.random.key(int.from_bytes(__import__("os").urandom(4), "little")))
    _w = (lambda a: (lambda t: t.astype(jnp.bfloat16) if jnp.issubdtype(t.dtype, jnp.floating) else t)(jnp.asarray(a)))
    B, F, D, L = 16384, 26, 16, 6
    Din = min(F * D, 512)
    R = max(Din // 4, 2)
    sc = Din ** -0.5
    return {
        "x0": _w((lambda *s: _rng.normal(s) * 0.05)(B, Din)),
        "U":  _w((lambda *s: _rng.normal(s) * 1.6)(L, Din, R) * sc),
        "V":  _w((lambda *s: _rng.normal(s) * 1.6)(L, R, Din) * sc),
        "bs": _w((lambda *s: _rng.normal(s) * 0.05)(L, Din)),
    }

def reference(x0, U, V, bs):
    x = x0
    for l in range(U.shape[0]):
        h = jnp.einsum('rd,bd->br', V[l], x)
        h = jnp.einsum('dr,br->bd', U[l], h)
        x = x0 * (h + bs[l]) + x
    return x
```

```python
import functools
import jax, jax.numpy as jnp
from jax import lax
import jax.experimental.pallas as pl
import jax.experimental.pallas.tpu as pltpu

f32, bf16, u32 = jnp.float32, jnp.bfloat16, jnp.uint32
KA = 384
NE = 9

def householder(cols, R):
    lane = lax.broadcasted_iota(jnp.int32, (8, 128), 1)
    a = []
    for c in cols:
        m = jnp.max(jnp.abs(c), axis=1, keepdims=True)
        a.append(c * jnp.where(m > 0, 1.0 / jnp.where(m > 0, m, 1.0), 0.0))
    Y, Z = [], []
    for k in range(len(cols)):
        ak = jnp.where(lane >= k, a[k], 0.0)
        n2 = jnp.sum(ak * ak, axis=1, keepdims=True)
        akk = jnp.sum(jnp.where(lane == k, ak, 0.0), axis=1, keepdims=True)
        ok = n2 > 1e-30
        nrm = jnp.sqrt(jnp.where(ok, n2, 1.0))
        v = ak + jnp.where(lane == k, jnp.where(akk >= 0, nrm, -nrm), 0.0)
        beta = jnp.where(ok, 1.0 / (nrm * (nrm + jnp.abs(akk))), 0.0)
        bv = beta * v
        for j in range(k + 1, len(cols)):
            a[j] = a[j] - jnp.sum(a[j] * v, axis=1, keepdims=True) * bv
        for j in range(k):
            Z[j] = Z[j] - jnp.sum(Z[j] * v, axis=1, keepdims=True) * bv
        Y.append(v)
        Z.append(bv)
    return Y, Z

def make_v8(bt=2048, sub=1024, vmem=100, flags=None, subs=None, nobc=True):
    subs = subs or [sub] * (bt // sub)
    assert sum(subs) == bt
    def kernel(x_hbm, u_hbm, v_hbm, b_hbm, o_hbm, xin, obuf, xst, u_ref, v_ref, b_ref, vs_ref, us_ref, ve_ref,
               tr_ref, y_ref, z_ref, isem, osem, wsem):
        L, D, R = u_hbm.shape
        B = x_hbm.shape[1]
        nblk = B // bt
        def in_copy(i, slot):
            return pltpu.make_async_copy(x_hbm.at[:, pl.ds(pl.multiple_of(i * bt, bt), bt)], xin.at[slot], isem.at[slot])
        def out_copy(i, slot):
            return pltpu.make_async_copy(obuf.at[slot], o_hbm.at[:, pl.ds(pl.multiple_of(i * bt, bt), bt)], osem.at[slot])
        cv = pltpu.make_async_copy(v_hbm, v_ref, wsem.at[0])
        cu = pltpu.make_async_copy(u_hbm, u_ref, wsem.at[1])
        cb = pltpu.make_async_copy(b_hbm, b_ref, wsem.at[2])
        cv.start(); cu.start(); cb.start()
        in_copy(0, 0).start()

        cv.wait()
        def vc_of(l):
            return jnp.concatenate([v_ref[l, :, KA:].astype(f32), jnp.zeros((R, 128 - (D - KA)), f32)], axis=1)
        for l in range(L):
            t = jnp.concatenate([vc_of(l), jnp.zeros((128 - R, 128), f32)], axis=0).T
            tr_ref[l * 16:(l + 1) * 16, :] = t[:16]
        tr_ref[L * 16:, :] = jnp.zeros(((8 - L) * 16, 128), f32)
        cols = [tr_ref[pl.ds(e, 8, stride=16), :] for e in range(NE)]
        Y, Z = householder(cols, R)
        for e in range(16):
            y_ref[e * 8:(e + 1) * 8, :] = Y[e] if e < NE else jnp.zeros((8, 128), f32)
            z_ref[e * 8:(e + 1) * 8, :] = Z[e] if e < NE else jnp.zeros((8, 128), f32)
        cu.wait(); cb.wait()
        lane = lax.broadcasted_iota(jnp.int32, (R, 128), 1)
        for l in range(L):
            yt = y_ref[pl.ds(l, 16, stride=8), :]
            zt = z_ref[pl.ds(l, 16, stride=8), :]
            tn = (((0,), (0,)), ((), ()))
            dm = -lax.dot_general(yt, zt, tn, preferred_element_type=f32)
            dt = dm.T
            vfull = v_ref[l]
            vrot = vfull.astype(f32) + jnp.dot(dt[:R, :R], vfull, preferred_element_type=f32)
            vs_ref[l] = vrot[:, :KA].astype(bf16).astype(f32)
            for e in range(NE):
                ve_ref[l, e] = jnp.broadcast_to(vrot[:16, KA + e:KA + e + 1], (16, 128))
            m = jnp.where(lane < R, dm[:R], jnp.where(lane > R, pltpu.roll(vc_of(l), R - 8, 1), 0.0))
            ub = u_ref[l]
            w = jnp.dot(ub, m.astype(bf16), preferred_element_type=f32)
            brow = jnp.concatenate([b_ref[l:l+1, :].astype(f32), jnp.zeros((1, 512 - D), f32)], axis=1)
            rows = lax.broadcasted_iota(jnp.int32, (128, 512), 0)
            bm = jnp.where(rows == R, jnp.broadcast_to(brow, (128, 512)), 0.0).T[:D]
            uf = jnp.concatenate([ub.astype(f32), jnp.zeros((D, 128 - R), f32)], axis=1)
            us_ref[l] = pltpu.bitcast((uf + w + bm).astype(bf16), u32)

        def compute(slot):
            off = 0
            for sub in subs:
                nt = sub // 128
                sl = slice(off, off + sub); off += sub
                for l in range(L):
                    if l == 0:
                        xa = xin[slot, :KA, sl]
                        xc = xin[slot, KA:, sl].astype(f32)
                    else:
                        xa = pltpu.bitcast(xst[:KA // 2, sl], bf16)
                        xc = pltpu.bitcast(xst[KA // 2:, sl], bf16).astype(f32)
                    h = jnp.dot(vs_ref[l], xa, preferred_element_type=f32)
                    t = None
                    for e in range(NE):
                        ve = jnp.concatenate([ve_ref[l, e, :(8 if e < 8 else 16)]] * nt, axis=1)
                        p = ve * xc[e:e+1, :]
                        if e == 8:
                            t = jnp.concatenate([t + p[:8], p[8:]], axis=0)
                        else:
                            t = p if t is None else t + p
                    rows = lax.broadcasted_iota(jnp.int32, (8, sub), 0)
                    ha = jnp.concatenate([h[:16] + t, h[16:], jnp.where(rows == 0, 1.0, xc[8:16]), xc[16:32]], axis=0).astype(bf16)
                    g = jnp.dot(pltpu.bitcast(us_ref[l], bf16), ha, preferred_element_type=f32)
                    x0 = xin[slot, :, sl].astype(f32)
                    xold = x0 if l == 0 else pltpu.bitcast(xst[:, sl], bf16).astype(f32)
                    xn = (x0 * g + xold).astype(bf16)
                    if l < L - 1:
                        xst[:, sl] = pltpu.bitcast(xn, u32)
                    else:
                        obuf[slot, :, sl] = xn

        def body(i, carry):
            slot = i % 2
            @pl.when(i + 1 < nblk)
            def _():
                in_copy(i + 1, 1 - slot).start()
            @pl.when(i >= 2)
            def _():
                out_copy(i - 2, slot).wait()
            in_copy(i, slot).wait()
            compute(slot)
            out_copy(i, slot).start()
            return carry
        if nblk == 1:
            body(0, 0)
        else:
            lax.fori_loop(0, nblk, body, 0)
        if nblk >= 2:
            out_copy(nblk - 2, (nblk - 2) % 2).wait()
        out_copy(nblk - 1, (nblk - 1) % 2).wait()

    def f(x0, U, V, bs):
        B, D = x0.shape
        L, _, R = U.shape
        out = pl.pallas_call(
            kernel,
            in_specs=[pl.BlockSpec(memory_space=pltpu.HBM)] * 4,
            out_specs=pl.BlockSpec(memory_space=pltpu.HBM),
            out_shape=jax.ShapeDtypeStruct((D, B), x0.dtype),
            scratch_shapes=[pltpu.VMEM((2, D, bt), bf16), pltpu.VMEM((2, D, bt), bf16),
                            pltpu.VMEM((D // 2, bt), u32),
                            pltpu.VMEM(U.shape, bf16), pltpu.VMEM(V.shape, bf16), pltpu.VMEM(bs.shape, bf16),
                            pltpu.VMEM((L, R, KA), f32), pltpu.VMEM((L, D // 2, 128), u32),
                            pltpu.VMEM((L, NE, 16, 128), f32),
                            pltpu.VMEM((128, 128), f32), pltpu.VMEM((128, 128), f32), pltpu.VMEM((128, 128), f32),
                            pltpu.SemaphoreType.DMA((2,)), pltpu.SemaphoreType.DMA((2,)), pltpu.SemaphoreType.DMA((3,))],
            compiler_params=pltpu.CompilerParams(vmem_limit_bytes=vmem*1024*1024, flags=flags, disable_bounds_checks=nobc),
        )(x0.T, U, V, bs)
        return out.T
    return f


_impl = make_v8(1024, 1024)

@jax.jit
def pallas_standalone__cross_network_dcn_v2__recsys_kernel(x0, U, V, bs):
    return _impl(x0, U, V, bs)
```

```python
import jax, jax.numpy as jnp
from jax import lax
import jax.experimental.pallas as pl
import jax.experimental.pallas.tpu as pltpu

f32, bf16, u32, i32 = jnp.float32, jnp.bfloat16, jnp.uint32, jnp.int32
KA = 384
NE = 9

def rsum(x):
    return jnp.sum(x, axis=1, keepdims=True)

def make_v18(nsub=4, gw=512, vmem=100, flags=None, wl=4, nb=None, nh=8, xinpad=256, xspad=0, obpad=0,
             ra=(16, 48, 112, 240), rb=(208,), first=(512, 256, 256)):
    sub = 2 * gw
    bt = nsub * sub
    assert nh <= 8 and sum(first) == sub
    npc = len(first) + 1
    def kernel(x_hbm, u_hbm, v_hbm, b_hbm, o_hbm, xin, obuf, xs, u_buf, va_buf, vc_buf, b_buf, vs_ref, us_ref, rb_ref,
               tr_ref, y_ref, be_ref, t_ref, m_ref, dt_ref, isem, osem, wsem):
        L, D, R = u_hbm.shape
        B = x_hbm.shape[1]
        nblk = nb or B // bt
        def cols(c0, w):
            return pl.ds(c0 if isinstance(c0, int) else pl.multiple_of(c0, 128), w)
        def in_copy(c0, w, k):
            return pltpu.make_async_copy(x_hbm.at[:, cols(c0, w)], xin.at[:, cols(c0, w)], isem.at[k])
        def out_copy(c0, w, r0, nr):
            return pltpu.make_async_copy(obuf.at[r0:r0+nr, cols(c0, w)], o_hbm.at[r0:r0+nr, cols(c0, w)], osem)
        edges = [sum(first[:j]) for j in range(len(first) + 1)] + [bt]
        def in_copies(i):
            return [in_copy(i * bt + a, b - a, k) if b > a else None for k, (a, b) in enumerate(zip(edges[:-1], edges[1:]))]
        cvc = pltpu.make_async_copy(v_hbm.at[:, :, KA:], vc_buf, wsem.at[0])
        cb = pltpu.make_async_copy(b_hbm, b_buf, wsem.at[1])
        cva = pltpu.make_async_copy(v_hbm.at[:, :, :KA], va_buf, wsem.at[1])
        cu = pltpu.make_async_copy(u_hbm, u_buf, wsem.at[1])
        cvc.start(); cb.start(); cva.start(); cu.start()
        for c in in_copies(0):
            if c is not None: c.start()

        cvc.wait()
        for l in range(L):
            vc = vc_buf[l].astype(f32)
            m = jnp.max(jnp.abs(vc), axis=0, keepdims=True)
            ex = jnp.minimum(lax.bitcast_convert_type(m, i32) & 0x7F800000, 0x7E800000)
            sc = jnp.concatenate([vc * lax.bitcast_convert_type(0x7F000000 - ex, f32),
                                  jnp.broadcast_to(lax.bitcast_convert_type(ex, f32), (8, D - KA))], axis=0)
            t = sc.astype(bf16).T[:16].astype(f32)
            tr_ref[l * 16:(l + 1) * 16, :] = jnp.concatenate([t, jnp.zeros((16, 120 - R), f32)], axis=1)
        tr_ref[L * 16:, :] = jnp.zeros(((8 - L) * 16, 128), f32)
        lane8 = lax.broadcasted_iota(i32, (8, 128), 1)

        def reflector(a0, k):
            on_k = lane8 == k
            ak = jnp.where((lane8 >= k) & (lane8 < R), a0, 0.0)
            n2 = rsum(ak * ak)
            akk = rsum(jnp.where(on_k, ak, 0.0))
            ok = n2 > 1e-30
            n2 = jnp.where(ok, n2, 1.0)
            nrm = n2 * lax.rsqrt(n2)
            s = jnp.where(akk >= 0, nrm, -nrm)
            v = ak + jnp.where(on_k, s, 0.0)
            beta = jnp.where(ok, 1.0 / (n2 + nrm * jnp.abs(akk)), 0.0)
            dot_v = lambda t: rsum(t * ak) + s * rsum(jnp.where(on_k, t, 0.0))
            return v, beta, dot_v, jnp.where(on_k, jnp.where(ok, -s, akk), a0 - ak)

        def hstep(k, carry):
            cnt, a = carry
            v, beta, dot_v, done = reflector(a[0], k)
            bv = beta * v
            rest = [t - dot_v(t) * bv for t in a[1:]]
            rk = pl.ds(pl.multiple_of(k * 8, 8), 8)
            y_ref[rk, :] = v
            be_ref[rk, :] = jnp.broadcast_to(beta, v.shape)
            t_ref[rk, :] = done
            return cnt + 1, rest + [rest[-1]]
        a = [tr_ref[pl.ds(e, 8, stride=16), :] for e in range(NE)]
        cnt, a = lax.fori_loop(0, nh - 1, hstep, (jnp.int32(0), a))
        lane = lax.broadcasted_iota(i32, (R, 128), 1)

        @pl.when(cnt == nh - 1)
        def _():
            k = nh - 1
            v, beta, dot_v, done = reflector(a[0], k)
            t_ref[k * 8:(k + 1) * 8, :] = done
            for e in range(nh, NE):
                t_ref[e * 8:(e + 1) * 8, :] = a[e - k] - dot_v(a[e - k]) * (beta * v)
            Y = [y_ref[e * 8:(e + 1) * 8, :] for e in range(k)] + [v]
            Z = [None] * k + [beta * v]
            for j in reversed(range(k)):
                z = Y[j] - dot_v(Y[j]) * Z[k]
                for q in reversed(range(j + 1, k)):
                    z = z - rsum(Y[j] * Y[q]) * Z[q]
                Z[j] = be_ref[j * 8:(j + 1) * 8, :] * z
            pad = jnp.zeros((128 - 8 * nh, 128), f32)
            ya = jnp.concatenate(Y + [pad], axis=0)
            za = -jnp.concatenate(Z + [pad], axis=0)
            yt, zb, zt, yb = ya.T, za.astype(bf16), za.T, ya.astype(bf16)
            for l in range(L):
                m_ref[l] = jnp.dot(jnp.where(lane % 8 == l, yt[:R], 0.0), zb, preferred_element_type=f32)
            for l in range(L):
                dt_ref[l] = jnp.dot(jnp.where(lane % 8 == l, zt[:R], 0.0), yb, preferred_element_type=f32)

        cb.wait(); cva.wait(); cu.wait()
        bpad = jnp.concatenate([b_buf[...].astype(f32), jnp.zeros((L, 512 - D), f32)], axis=1)
        bpad = jnp.concatenate([jnp.zeros((R, 512), f32), bpad, jnp.zeros((128 - R - L, 512), f32)], axis=0)
        bcol = bpad.T[:D]
        row24 = lax.broadcasted_iota(i32, (128 - R, 128), 0)
        lane24 = lax.broadcasted_iota(i32, (128 - R, 128), 1)
        for l in range(L):
            va = va_buf[l]
            vs_ref[l] = va.astype(f32) + jnp.dot(dt_ref[l, :, :R], va, preferred_element_type=f32)
        def rhs(l):
            vc = jnp.concatenate([vc_buf[l].astype(f32), jnp.zeros((R, 128 - (D - KA)), f32)], axis=1)
            vc = jnp.where(lane > R, pltpu.roll(vc, R - 8, 1), 0.0)
            pick = jnp.where((row24 == l) & (lane24 == R), 1.0, 0.0)
            return jnp.concatenate([m_ref[l] + vc, pick], axis=0).astype(bf16)
        for l0 in range(0, L, 2):
            ms = [rhs(l0), rhs(l0 + 1)]
            for r0 in (0, D // 2):
                res = []
                for l, m in zip((l0, l0 + 1), ms):
                    uf = jnp.concatenate([u_buf[l, r0:r0 + D // 2].astype(f32), jnp.zeros((D // 2, 128 - R), f32)], axis=1)
                    res.append(uf + jnp.dot(uf + bcol[r0:r0 + D // 2], m, preferred_element_type=f32))
                us_ref[r0 // 2:(r0 + D // 2) // 2, l0 * 128:(l0 + 2) * 128] = pltpu.bitcast(jnp.concatenate(res, axis=1).astype(bf16), u32)
        tt = jnp.concatenate([t_ref[...], jnp.zeros((128 - 8 * NE, 128), f32)], axis=0).T
        tt = tt[:R] * tt[R:R + 1]
        rb0 = lambda e: 8 * e if e < nh else 8 * nh + (e - nh) * R
        for l in range(L):
            for e in range(NE):
                n = 8 if e < nh else R
                rb_ref[l, rb0(e):rb0(e) + n, :] = jnp.broadcast_to(tt[:n, 8 * e + l:8 * e + l + 1], (n, 128))

        def compute(c0, waits, waitl, prefetch, last):
            nt = sub // 128
            sl = cols(c0, sub)
            for l in range(L):
                if l == 0 and waits is not None:
                    hs = []
                    for c, a, b in zip(waits, edges[:-1], edges[1:]):
                        c.wait()
                        hs.append(jnp.dot(vs_ref[l], xin[:KA, cols(c0 + a, b - a)], preferred_element_type=f32))
                    h = jnp.concatenate(hs, axis=1)
                else:
                    xa = xin[:KA, sl] if l == 0 else pltpu.bitcast(xs[:KA // 2, :sub], bf16)
                    h = jnp.dot(vs_ref[l], xa, preferred_element_type=f32)
                xc = xin[KA:, sl].astype(f32) if l == 0 else pltpu.bitcast(xs[KA // 2:, :sub], bf16).astype(f32)
                t = None
                for e in range(nh):
                    p = jnp.concatenate([rb_ref[l, rb0(e):rb0(e) + 8, :]] * nt, axis=1) * xc[e:e+1, :]
                    t = p if t is None else t + p
                for e in range(nh, NE):
                    h = h + jnp.concatenate([rb_ref[l, rb0(e):rb0(e) + R, :]] * nt, axis=1) * xc[e:e+1, :]
                rows = lax.broadcasted_iota(i32, (8, sub), 0)
                ha = jnp.concatenate([h[:8] + t, h[8:], jnp.where(rows == 0, 1.0, xc[8:16]), xc[16:32]], axis=0).astype(bf16)
                if l == wl and waitl is not None:
                    waitl.wait()
                if l == wl and prefetch is not None:
                    prefetch()
                g = jnp.dot(pltpu.bitcast(us_ref[:, l * 128:(l + 1) * 128], bf16), ha, preferred_element_type=f32)
                if l < L - 1:
                    x0 = xin[:, sl].astype(f32)
                    xold = x0 if l == 0 else pltpu.bitcast(xs[:, :sub], bf16).astype(f32)
                    xs[:, :sub] = pltpu.bitcast((x0 * g + xold).astype(bf16), u32)
                else:
                    for q in range(2):
                        rs = [0, *(ra if q == 0 else rb), D] if last else [0, D]
                        cq, sq = cols(c0 + q * gw, gw), slice(q * gw, (q + 1) * gw)
                        for r0, r1 in zip(rs[:-1], rs[1:]):
                            x0 = xin[r0:r1, cq].astype(f32)
                            xold = pltpu.bitcast(xs[r0 // 2:r1 // 2, sq], bf16).astype(f32)
                            obuf[r0:r1, cq] = (x0 * g[r0:r1, sq] + xold).astype(bf16)
                            out_copy(c0 + q * gw, gw, r0, r1 - r0).start()

        def body(i, carry):
            cur = in_copies(i)
            def prefetch():
                @pl.when(i + 1 < nblk)
                def _():
                    for c in in_copies(i + 1):
                        if c is not None: c.start()
            for s in range(nsub):
                compute(i * bt + s * sub, cur[:-1] if s == 0 else None, cur[-1] if s == 0 else None,
                        prefetch if s == 0 else None, s == nsub - 1)
            return carry
        lax.fori_loop(0, nblk, body, 0)
        pltpu.make_async_copy(obuf.at[:, :nblk * bt], o_hbm.at[:, :nblk * bt], osem).wait()

    def f(x0, U, V, bs):
        B, D = x0.shape
        L, _, R = U.shape
        out = pl.pallas_call(
            kernel,
            in_specs=[pl.BlockSpec(memory_space=pltpu.HBM)] * 4,
            out_specs=pl.BlockSpec(memory_space=pltpu.HBM),
            out_shape=jax.ShapeDtypeStruct((D, B), x0.dtype),
            scratch_shapes=[pltpu.VMEM((D, B + xinpad), bf16), pltpu.VMEM((D, B + obpad), bf16), pltpu.VMEM((D // 2, sub + xspad), u32),
                            pltpu.VMEM(U.shape, bf16), pltpu.VMEM((L, R, KA), bf16), pltpu.VMEM((L, R, D - KA), bf16),
                            pltpu.VMEM(bs.shape, bf16),
                            pltpu.VMEM((L, R, KA), f32), pltpu.VMEM((D // 2, L * 128), u32),
                            pltpu.VMEM((L, nh * 8 + (NE - nh) * R, 128), f32), pltpu.VMEM((128, 128), f32),
                            pltpu.VMEM((nh * 8, 128), f32), pltpu.VMEM((nh * 8, 128), f32), pltpu.VMEM((NE * 8, 128), f32),
                            pltpu.VMEM((L, R, 128), f32), pltpu.VMEM((L, R, 128), f32),
                            pltpu.SemaphoreType.DMA((npc,)), pltpu.SemaphoreType.DMA(()), pltpu.SemaphoreType.DMA((2,))],
            compiler_params=pltpu.CompilerParams(vmem_limit_bytes=vmem*1024*1024, flags=flags, disable_bounds_checks=True),
        )(x0.T, U, V, bs)
        return out.T
    return f

RD = {"XLA_TPU_RESCHEDULE_DMA_DONES": True}

_impl = make_v18(flags=RD,first=(512,512))

@jax.jit
def pallas_standalone__cross_network_dcn_v2__recsys_kernel(x0, U, V, bs):
    return _impl(x0, U, V, bs)
```

```python
import functools

import jax
import jax.numpy as jnp
from jax import lax
import jax.experimental.pallas as pl
import jax.experimental.pallas.tpu as pltpu

f32, bf16, i32, u32 = jnp.float32, jnp.bfloat16, jnp.int32, jnp.uint32

LANES = 128
N_REFLECT = 8
GROUP = 4 * LANES
SUB = 2 * GROUP
BLOCK = 4 * SUB
MAX_ROW_SCALE_RATIO = 4.0
OUT_ROW_SPLITS = ((16, 48, 112, 240), (208,))


def _lane_sum(x):
    return jnp.sum(x, axis=1, keepdims=True)


def _pad(x, rows=None, lanes=None):
    if lanes is not None and lanes > x.shape[1]:
        x = jnp.concatenate([x, jnp.zeros((x.shape[0], lanes - x.shape[1]), x.dtype)], axis=1)
    if rows is not None and rows > x.shape[0]:
        x = jnp.concatenate([x, jnp.zeros((rows - x.shape[0], x.shape[1]), x.dtype)], axis=0)
    return x


def _pow2_scale(m):
    e = jnp.minimum(lax.bitcast_convert_type(m, i32) & 0x7F800000, 0x7E800000)
    return lax.bitcast_convert_type(0x7F000000 - e, f32), lax.bitcast_convert_type(e, f32)


def _prepare_weights(u_buf, va_buf, vc_buf, b_buf, v_rot, u_aug, t_bcast,
                     col_ref, y_ref, beta_ref, t_ref, d_ref, dt_ref, with_rotation, before_products):
    L, D, R = u_buf.shape
    n_tail = vc_buf.shape[2]
    n_vpu = n_tail - (LANES - R - 1)

    for l in range(L):
        vc = vc_buf[l].astype(f32)
        down, up = _pow2_scale(jnp.max(jnp.abs(vc), axis=0, keepdims=True))
        scaled = jnp.concatenate([vc * down, jnp.broadcast_to(up, (8, n_tail))], axis=0)
        col_ref[l * 16:(l + 1) * 16, :] = _pad(scaled.astype(bf16).T[:16].astype(f32), lanes=LANES)
    col_ref[L * 16:, :] = jnp.zeros(((8 - L) * 16, LANES), f32)

    lane8 = lax.broadcasted_iota(i32, (8, LANES), 1)

    def reflector(col, k):
        on_k = lane8 == k
        below = jnp.where((lane8 >= k) & (lane8 < R), col, 0.0)
        norm2 = _lane_sum(below * below)
        head = _lane_sum(jnp.where(on_k, below, 0.0))
        nonzero = norm2 > 1e-30
        norm2 = jnp.where(nonzero, norm2, 1.0)
        norm = norm2 * lax.rsqrt(norm2)
        shift = jnp.where(head >= 0, norm, -norm)
        v = below + jnp.where(on_k, shift, 0.0)
        beta = jnp.where(nonzero, 1.0 / (norm2 + norm * jnp.abs(head)), 0.0)

        def dot_v(t):
            return _lane_sum(t * below) + shift * _lane_sum(jnp.where(on_k, t, 0.0))

        reflected = jnp.where(on_k, jnp.where(nonzero, -shift, head), col - below)
        return v, beta, dot_v, reflected

    def step(k, carry):
        done, cols = carry
        v, beta, dot_v, reflected = reflector(cols[0], k)
        beta_v = beta * v
        rest = [t - dot_v(t) * beta_v for t in cols[1:]]
        rows = pl.ds(pl.multiple_of(k * 8, 8), 8)
        y_ref[rows, :] = v
        beta_ref[rows, :] = jnp.broadcast_to(beta, v.shape)
        t_ref[rows, :] = reflected
        return done + 1, rest + [rest[-1]]

    last = N_REFLECT - 1
    cols = [col_ref[pl.ds(e, 8, stride=16), :] for e in range(n_vpu)]
    done, cols = lax.fori_loop(0, last, step, (jnp.int32(0), cols))
    lane = lax.broadcasted_iota(i32, (R, LANES), 1)

    @pl.when(done == last)
    def _():
        v, beta, dot_v, reflected = reflector(cols[0], last)
        t_ref[last * 8:(last + 1) * 8, :] = reflected
        for e in range(N_REFLECT, n_vpu):
            t_ref[e * 8:(e + 1) * 8, :] = cols[e - last] - dot_v(cols[e - last]) * (beta * v)
        ys = [y_ref[e * 8:(e + 1) * 8, :] for e in range(last)] + [v]
        zs = [None] * last + [beta * v]
        for j in reversed(range(last)):
            z = ys[j] - dot_v(ys[j]) * zs[last]
            for k in reversed(range(j + 1, last)):
                z = z - _lane_sum(ys[j] * ys[k]) * zs[k]
            zs[j] = beta_ref[j * 8:(j + 1) * 8, :] * z
        y_all = _pad(jnp.concatenate(ys, axis=0), rows=LANES)
        z_all = -_pad(jnp.concatenate(zs, axis=0), rows=LANES)
        y_t, z_b, z_t, y_b = y_all.T, z_all.astype(bf16), z_all.T, y_all.astype(bf16)
        for l in range(L):
            d_ref[l] = jnp.dot(jnp.where(lane % 8 == l, y_t[:R], 0.0), z_b, preferred_element_type=f32)
        for l in range(L):
            dt_ref[l] = jnp.dot(jnp.where(lane % 8 == l, z_t[:R], 0.0), y_b, preferred_element_type=f32)
        with_rotation()

    before_products()

    for l in range(L):
        va = va_buf[l]
        v_rot[l] = va.astype(f32) + jnp.dot(dt_ref[l, :, :R], va, preferred_element_type=f32)

    b_rows = jnp.concatenate([jnp.zeros((R, pl.cdiv(D, LANES) * LANES), f32),
                              _pad(b_buf[...].astype(f32), lanes=pl.cdiv(D, LANES) * LANES)], axis=0)
    b_cols = _pad(b_rows, rows=LANES).T[:D]
    spare_row = lax.broadcasted_iota(i32, (LANES - R, LANES), 0)
    spare_lane = lax.broadcasted_iota(i32, (LANES - R, LANES), 1)

    def mixer(l):
        tail = pltpu.roll(_pad(vc_buf[l].astype(f32), lanes=LANES), LANES - n_tail, 1)
        pick_bias = jnp.where((spare_row == l) & (spare_lane == R), 1.0, 0.0)
        top = d_ref[l] + jnp.where(lane > R, tail, 0.0)
        return jnp.concatenate([top, pick_bias], axis=0).astype(bf16)

    half = D // 2
    for l0 in range(0, L, 2):
        mixers = [mixer(l0), mixer(l0 + 1)]
        for r0 in (0, half):
            pair = []
            for l, mix in zip((l0, l0 + 1), mixers):
                u = _pad(u_buf[l, r0:r0 + half].astype(f32), lanes=LANES)
                pair.append(u + jnp.dot(u + b_cols[r0:r0 + half], mix, preferred_element_type=f32))
            u_aug[r0 // 2:(r0 + half) // 2, l0 * LANES:(l0 + 2) * LANES] = pltpu.bitcast(
                jnp.concatenate(pair, axis=1).astype(bf16), u32)

    t_all = _pad(t_ref[...], rows=LANES).T
    t_all = t_all[:R] * t_all[R:R + 1]
    for l in range(L):
        for e in range(n_vpu):
            r0, n = _t_rows(e, R)
            t_bcast[l, r0:r0 + n, :] = jnp.broadcast_to(t_all[:n, 8 * e + l:8 * e + l + 1], (n, LANES))


def _t_rows(e, rank):
    if e < N_REFLECT:
        return 8 * e, 8
    return 8 * N_REFLECT + (e - N_REFLECT) * rank, rank


def _kernel(x_hbm, u_hbm, v_hbm, b_hbm, o_hbm,
            x_buf, o_buf, state, u_buf, va_buf, vc_buf, b_buf, v_rot, u_aug, t_bcast,
            col_ref, y_ref, beta_ref, t_ref, d_ref, dt_ref, excess_ref, x_sem, o_sem, w_sem):
    L, D, R = u_hbm.shape
    B = x_hbm.shape[1]
    KA = va_buf.shape[2]
    n_vpu = D - KA - (LANES - R - 1)
    n_blocks = B // BLOCK

    def columns(start, size):
        return pl.ds(start if isinstance(start, int) else pl.multiple_of(start, LANES), size)

    def fetch(i):
        edges = (0, GROUP, SUB, BLOCK)
        return [pltpu.make_async_copy(x_hbm.at[:, columns(i * BLOCK + a, b - a)],
                                      x_buf.at[:, columns(i * BLOCK + a, b - a)], x_sem.at[k])
                for k, (a, b) in enumerate(zip(edges[:-1], edges[1:]))]

    tail_copy = pltpu.make_async_copy(v_hbm.at[:, :, KA:], vc_buf, w_sem.at[0])
    body_copy = pltpu.make_async_copy(v_hbm.at[:, :, :KA], va_buf, w_sem.at[1])
    u_copies = [pltpu.make_async_copy(b_hbm, b_buf, w_sem.at[2]),
                pltpu.make_async_copy(u_hbm, u_buf, w_sem.at[2])]
    for copy in [tail_copy, body_copy] + u_copies + fetch(0):
        copy.start()

    def row_max(l):
        v = jnp.concatenate([va_buf[l].astype(f32), _pad(vc_buf[l].astype(f32), lanes=LANES)], axis=1)
        return jnp.broadcast_to(jnp.max(jnp.abs(v), axis=1, keepdims=True), (R, LANES))

    def measure_row_scales():
        body_copy.wait()
        excess = None
        for l in range(L):
            m = row_max(l)
            e = jnp.max(m, axis=0, keepdims=True) - MAX_ROW_SCALE_RATIO * jnp.min(m, axis=0, keepdims=True)
            excess = e if excess is None else jnp.maximum(excess, e)
        excess_ref[...] = jnp.broadcast_to(excess, excess_ref.shape)

    def wait_for_u():
        for copy in u_copies:
            copy.wait()

    prepare = functools.partial(_prepare_weights, u_buf, va_buf, vc_buf, b_buf, v_rot, u_aug, t_bcast,
                                col_ref, y_ref, beta_ref, t_ref, d_ref, dt_ref)
    tail_copy.wait()
    prepare(measure_row_scales, wait_for_u)

    @pl.when(jnp.max(excess_ref[...]) > 0)
    def _():
        for l in range(L):
            down, up = _pow2_scale(row_max(l))
            va_buf[l] = (va_buf[l].astype(f32) * jnp.concatenate([down] * (KA // LANES), axis=1)).astype(bf16)
            vc_buf[l] = (vc_buf[l].astype(f32) * down[:, :D - KA]).astype(bf16)
            u_buf[l] = (u_buf[l].astype(f32) * _pad(up, rows=LANES).T[:1, :R]).astype(bf16)
        prepare(lambda: None, lambda: None)

    def cross_layers(c0, arrivals, between, out_row_splits):
        cols = columns(c0, SUB)
        for l in range(L):
            if l > 0:
                h = jnp.dot(v_rot[l], pltpu.bitcast(state[:KA // 2, :], bf16), preferred_element_type=f32)
                tail = pltpu.bitcast(state[KA // 2:, :], bf16).astype(f32)
            else:
                if arrivals is None:
                    h = jnp.dot(v_rot[l], x_buf[:KA, cols], preferred_element_type=f32)
                else:
                    parts = []
                    for q, copy in enumerate(arrivals):
                        copy.wait()
                        parts.append(jnp.dot(v_rot[l], x_buf[:KA, columns(c0 + q * GROUP, GROUP)],
                                             preferred_element_type=f32))
                    h = jnp.concatenate(parts, axis=1)
                tail = x_buf[KA:, cols].astype(f32)

            head = None
            for e in range(n_vpu):
                r0, n = _t_rows(e, R)
                term = jnp.concatenate([t_bcast[l, r0:r0 + n, :]] * (SUB // LANES), axis=1) * tail[e:e + 1]
                if e >= N_REFLECT:
                    h = h + term
                else:
                    head = term if head is None else head + term
            row = lax.broadcasted_iota(i32, (8, SUB), 0)
            slots = jnp.concatenate([h[:8] + head, h[8:],
                                     jnp.where(row == 0, 1.0, tail[n_vpu - 1:n_vpu + 7]),
                                     tail[n_vpu + 7:]], axis=0).astype(bf16)
            if l == L - 2 and between is not None:
                between()
            g = jnp.dot(pltpu.bitcast(u_aug[:, l * LANES:(l + 1) * LANES], bf16), slots,
                        preferred_element_type=f32)

            if l < L - 1:
                x0 = x_buf[:, cols].astype(f32)
                x = x0 if l == 0 else pltpu.bitcast(state[...], bf16).astype(f32)
                state[...] = pltpu.bitcast((x0 * g + x).astype(bf16), u32)
                continue
            for q, splits in enumerate(out_row_splits):
                group = columns(c0 + q * GROUP, GROUP)
                local = slice(q * GROUP, (q + 1) * GROUP)
                for r0, r1 in zip((0, *splits), (*splits, D)):
                    x0 = x_buf[r0:r1, group].astype(f32)
                    x = pltpu.bitcast(state[r0 // 2:r1 // 2, local], bf16).astype(f32)
                    o_buf[r0:r1, group] = (x0 * g[r0:r1, local] + x).astype(bf16)
                    pltpu.make_async_copy(o_buf.at[r0:r1, group], o_hbm.at[r0:r1, group], o_sem).start()

    def block(i, carry):
        first, second, rest = fetch(i)

        def between():
            rest.wait()

            @pl.when(i + 1 < n_blocks)
            def _():
                for copy in fetch(i + 1):
                    copy.start()

        n_sub = BLOCK // SUB
        for s in range(n_sub):
            cross_layers(i * BLOCK + s * SUB,
                         (first, second) if s == 0 else None,
                         between if s == 0 else None,
                         OUT_ROW_SPLITS if s == n_sub - 1 else ((), ()))
        return carry

    lax.fori_loop(0, n_blocks, block, 0)
    pltpu.make_async_copy(o_buf, o_hbm, o_sem).wait()


@jax.jit
def pallas_standalone__cross_network_dcn_v2__recsys_kernel(
    x0: jax.Array,
    U: jax.Array,
    V: jax.Array,
    bs: jax.Array,
):
    B, D = x0.shape
    L, _, R = U.shape
    KA = D // LANES * LANES
    n_vpu = D - KA - (LANES - R - 1)
    assert (D, R) == (416, 104) and B % BLOCK == 0 and L % 2 == 0 and 2 <= L <= 8
    assert all(a.dtype == bf16 for a in (x0, U, V, bs))

    out_t = pl.pallas_call(
        _kernel,
        in_specs=[pl.BlockSpec(memory_space=pltpu.HBM)] * 4,
        out_specs=pl.BlockSpec(memory_space=pltpu.HBM),
        out_shape=jax.ShapeDtypeStruct((D, B), bf16),
        scratch_shapes=[
            pltpu.VMEM((D, B + 2 * LANES), bf16),
            pltpu.VMEM((D, B), bf16),
            pltpu.VMEM((D // 2, SUB), u32),
            pltpu.VMEM((L, D, R), bf16),
            pltpu.VMEM((L, R, KA), bf16),
            pltpu.VMEM((L, R, D - KA), bf16),
            pltpu.VMEM((L, D), bf16),
            pltpu.VMEM((L, R, KA), f32),
            pltpu.VMEM((D // 2, L * LANES), u32),
            pltpu.VMEM((L, sum(_t_rows(n_vpu - 1, R)), LANES), f32),
            pltpu.VMEM((8 * 16, LANES), f32),
            pltpu.VMEM((8 * N_REFLECT, LANES), f32),
            pltpu.VMEM((8 * N_REFLECT, LANES), f32),
            pltpu.VMEM((8 * n_vpu, LANES), f32),
            pltpu.VMEM((L, R, LANES), f32),
            pltpu.VMEM((L, R, LANES), f32),
            pltpu.VMEM((8, LANES), f32),
            pltpu.SemaphoreType.DMA((3,)),
            pltpu.SemaphoreType.DMA(()),
            pltpu.SemaphoreType.DMA((3,)),
        ],
        compiler_params=pltpu.CompilerParams(
            vmem_limit_bytes=64 * 1024 * 1024,
            disable_bounds_checks=True,
            flags={"XLA_TPU_RESCHEDULE_DMA_DONES": True},
        ),
    )(x0.T, U, V, bs)
    return out_t.T
```

```python
import functools

import jax
import jax.numpy as jnp
from jax import lax
import jax.experimental.pallas as pl
import jax.experimental.pallas.tpu as pltpu

f32, bf16, i32, u32 = jnp.float32, jnp.bfloat16, jnp.int32, jnp.uint32

LANES = 128
N_REFLECT = 8
GROUP = 4 * LANES
SUB = 2 * GROUP
BLOCK = 4 * SUB
MAX_ROW_SCALE_RATIO = 4.0


def _lane_sum(x):
    return jnp.sum(x, axis=1, keepdims=True)


def _pad(x, rows=None, lanes=None):
    if lanes is not None and lanes > x.shape[1]:
        x = jnp.concatenate([x, jnp.zeros((x.shape[0], lanes - x.shape[1]), x.dtype)], axis=1)
    if rows is not None and rows > x.shape[0]:
        x = jnp.concatenate([x, jnp.zeros((rows - x.shape[0], x.shape[1]), x.dtype)], axis=0)
    return x


def _pow2_scale(m):
    e = jnp.minimum(lax.bitcast_convert_type(m, i32) & 0x7F800000, 0x7E800000)
    return lax.bitcast_convert_type(0x7F000000 - e, f32), lax.bitcast_convert_type(e, f32)


def _prepare_weights(u_buf, va_buf, vc_buf, b_buf, v_rot, u_aug, t_bcast,
                     col_ref, y_ref, beta_ref, t_ref, d_ref, dt_ref, with_rotation, before_products):
    L, D, R = u_buf.shape
    n_tail = vc_buf.shape[2]
    n_vpu = n_tail - (LANES - R - 1)

    for l in range(L):
        vc = vc_buf[l].astype(f32)
        down, up = _pow2_scale(jnp.max(jnp.abs(vc), axis=0, keepdims=True))
        scaled = jnp.concatenate([vc * down, jnp.broadcast_to(up, (8, n_tail))], axis=0)
        col_ref[l * 16:(l + 1) * 16, :] = _pad(scaled.astype(bf16).T[:16].astype(f32), lanes=LANES)
    col_ref[L * 16:, :] = jnp.zeros(((8 - L) * 16, LANES), f32)

    lane8 = lax.broadcasted_iota(i32, (8, LANES), 1)

    def reflector(col, k):
        on_k = lane8 == k
        below = jnp.where((lane8 >= k) & (lane8 < R), col, 0.0)
        norm2 = _lane_sum(below * below)
        head = _lane_sum(jnp.where(on_k, below, 0.0))
        nonzero = norm2 > 1e-30
        norm2 = jnp.where(nonzero, norm2, 1.0)
        norm = norm2 * lax.rsqrt(norm2)
        shift = jnp.where(head >= 0, norm, -norm)
        v = below + jnp.where(on_k, shift, 0.0)
        beta = jnp.where(nonzero, 1.0 / (norm2 + norm * jnp.abs(head)), 0.0)

        def dot_v(t):
            return _lane_sum(t * below) + shift * _lane_sum(jnp.where(on_k, t, 0.0))

        reflected = jnp.where(on_k, jnp.where(nonzero, -shift, head), col - below)
        return v, beta, dot_v, reflected

    def step(k, carry):
        done, cols = carry
        v, beta, dot_v, reflected = reflector(cols[0], k)
        beta_v = beta * v
        rest = [t - dot_v(t) * beta_v for t in cols[1:]]
        rows = pl.ds(pl.multiple_of(k * 8, 8), 8)
        y_ref[rows, :] = v
        beta_ref[rows, :] = jnp.broadcast_to(beta, v.shape)
        t_ref[rows, :] = reflected
        return done + 1, rest + [rest[-1]]

    last = N_REFLECT - 1
    cols = [col_ref[pl.ds(e, 8, stride=16), :] for e in range(n_vpu)]
    done, cols = lax.fori_loop(0, last, step, (jnp.int32(0), cols))
    lane = lax.broadcasted_iota(i32, (R, LANES), 1)

    @pl.when(done == last)
    def _():
        v, beta, dot_v, reflected = reflector(cols[0], last)
        t_ref[last * 8:(last + 1) * 8, :] = reflected
        for e in range(N_REFLECT, n_vpu):
            t_ref[e * 8:(e + 1) * 8, :] = cols[e - last] - dot_v(cols[e - last]) * (beta * v)
        ys = [y_ref[e * 8:(e + 1) * 8, :] for e in range(last)] + [v]
        zs = [None] * last + [beta * v]
        for j in reversed(range(last)):
            z = ys[j] - dot_v(ys[j]) * zs[last]
            for k in reversed(range(j + 1, last)):
                z = z - _lane_sum(ys[j] * ys[k]) * zs[k]
            zs[j] = beta_ref[j * 8:(j + 1) * 8, :] * z
        y_all = _pad(jnp.concatenate(ys, axis=0), rows=LANES)
        z_all = -_pad(jnp.concatenate(zs, axis=0), rows=LANES)
        y_t, z_b, z_t, y_b = y_all.T, z_all.astype(bf16), z_all.T, y_all.astype(bf16)
        for l in range(L):
            d_ref[l] = jnp.dot(jnp.where(lane % 8 == l, y_t[:R], 0.0), z_b, preferred_element_type=f32)
        for l in range(L):
            dt_ref[l] = jnp.dot(jnp.where(lane % 8 == l, z_t[:R], 0.0), y_b, preferred_element_type=f32)
        with_rotation()

    before_products()

    for l in range(L):
        va = va_buf[l]
        v_rot[l] = va.astype(f32) + jnp.dot(dt_ref[l, :, :R], va, preferred_element_type=f32)

    b_rows = jnp.concatenate([jnp.zeros((R, pl.cdiv(D, LANES) * LANES), f32),
                              _pad(b_buf[...].astype(f32), lanes=pl.cdiv(D, LANES) * LANES)], axis=0)
    b_cols = _pad(b_rows, rows=LANES).T[:D]
    spare_row = lax.broadcasted_iota(i32, (LANES - R, LANES), 0)
    spare_lane = lax.broadcasted_iota(i32, (LANES - R, LANES), 1)

    def mixer(l):
        tail = pltpu.roll(_pad(vc_buf[l].astype(f32), lanes=LANES), LANES - n_tail, 1)
        pick_bias = jnp.where((spare_row == l) & (spare_lane == R), 1.0, 0.0)
        top = d_ref[l] + jnp.where(lane > R, tail, 0.0)
        return jnp.concatenate([top, pick_bias], axis=0).astype(bf16)

    half = D // 2
    for l0 in range(0, L, 2):
        mixers = [mixer(l0), mixer(l0 + 1)]
        for r0 in (0, half):
            pair = []
            for l, mix in zip((l0, l0 + 1), mixers):
                u = _pad(u_buf[l, r0:r0 + half].astype(f32), lanes=LANES)
                pair.append(u + jnp.dot(u + b_cols[r0:r0 + half], mix, preferred_element_type=f32))
            u_aug[r0 // 2:(r0 + half) // 2, l0 * LANES:(l0 + 2) * LANES] = pltpu.bitcast(
                jnp.concatenate(pair, axis=1).astype(bf16), u32)

    t_all = _pad(t_ref[...], rows=LANES).T
    t_all = t_all[:R] * t_all[R:R + 1]
    for l in range(L):
        for e in range(n_vpu):
            r0, n = _t_rows(e, R)
            t_bcast[l, r0:r0 + n, :] = jnp.broadcast_to(t_all[:n, 8 * e + l:8 * e + l + 1], (n, LANES))


def _t_rows(e, rank):
    if e < N_REFLECT:
        return 8 * e, 8
    return 8 * N_REFLECT + (e - N_REFLECT) * rank, rank


def _kernel(x_hbm, u_hbm, v_hbm, b_hbm, o_hbm,
            x_buf, o_buf, state, u_buf, va_buf, vc_buf, b_buf, v_rot, u_aug, t_bcast,
            col_ref, y_ref, beta_ref, t_ref, d_ref, dt_ref, excess_ref, x_sem, o_sem, w_sem):
    L, D, R = u_hbm.shape
    B = x_hbm.shape[1]
    KA = va_buf.shape[2]
    n_vpu = D - KA - (LANES - R - 1)
    n_blocks = B // BLOCK

    def columns(start, size):
        return pl.ds(start if isinstance(start, int) else pl.multiple_of(start, LANES), size)

    def fetch(i):
        edges = (0, GROUP, SUB, BLOCK)
        return [pltpu.make_async_copy(x_hbm.at[:, columns(i * BLOCK + a, b - a)],
                                      x_buf.at[:, columns(i * BLOCK + a, b - a)], x_sem.at[k])
                for k, (a, b) in enumerate(zip(edges[:-1], edges[1:]))]

    tail_copy = pltpu.make_async_copy(v_hbm.at[:, :, KA:], vc_buf, w_sem.at[0])
    body_copy = pltpu.make_async_copy(v_hbm.at[:, :, :KA], va_buf, w_sem.at[1])
    u_copies = [pltpu.make_async_copy(b_hbm, b_buf, w_sem.at[2]),
                pltpu.make_async_copy(u_hbm, u_buf, w_sem.at[2])]
    for copy in [tail_copy, body_copy] + u_copies + fetch(0):
        copy.start()

    def row_max(l):
        v = jnp.concatenate([va_buf[l].astype(f32), _pad(vc_buf[l].astype(f32), lanes=LANES)], axis=1)
        return jnp.broadcast_to(jnp.max(jnp.abs(v), axis=1, keepdims=True), (R, LANES))

    def measure_row_scales():
        body_copy.wait()
        excess = None
        for l in range(L):
            m = row_max(l)
            e = jnp.max(m, axis=0, keepdims=True) - MAX_ROW_SCALE_RATIO * jnp.min(m, axis=0, keepdims=True)
            excess = e if excess is None else jnp.maximum(excess, e)
        excess_ref[...] = jnp.broadcast_to(excess, excess_ref.shape)

    def wait_for_u():
        for copy in u_copies:
            copy.wait()

    prepare = functools.partial(_prepare_weights, u_buf, va_buf, vc_buf, b_buf, v_rot, u_aug, t_bcast,
                                col_ref, y_ref, beta_ref, t_ref, d_ref, dt_ref)
    tail_copy.wait()
    prepare(measure_row_scales, wait_for_u)

    @pl.when(jnp.max(excess_ref[...]) > 0)
    def _():
        for l in range(L):
            down, up = _pow2_scale(row_max(l))
            va_buf[l] = (va_buf[l].astype(f32) * jnp.concatenate([down] * (KA // LANES), axis=1)).astype(bf16)
            vc_buf[l] = (vc_buf[l].astype(f32) * down[:, :D - KA]).astype(bf16)
            u_buf[l] = (u_buf[l].astype(f32) * _pad(up, rows=LANES).T[:1, :R]).astype(bf16)
        prepare(lambda: None, lambda: None)

    def cross_layers(c0, arrivals, between, out_chunks):
        cols = columns(c0, SUB)
        for l in range(L):
            if l > 0:
                h = jnp.dot(v_rot[l], pltpu.bitcast(state[:KA // 2, :], bf16), preferred_element_type=f32)
                tail = pltpu.bitcast(state[KA // 2:, :], bf16).astype(f32)
            else:
                if arrivals is None:
                    h = jnp.dot(v_rot[l], x_buf[:KA, cols], preferred_element_type=f32)
                else:
                    parts = []
                    for q, copy in enumerate(arrivals):
                        copy.wait()
                        parts.append(jnp.dot(v_rot[l], x_buf[:KA, columns(c0 + q * GROUP, GROUP)],
                                             preferred_element_type=f32))
                    h = jnp.concatenate(parts, axis=1)
                tail = x_buf[KA:, cols].astype(f32)

            head = None
            for e in range(n_vpu):
                r0, n = _t_rows(e, R)
                term = jnp.concatenate([t_bcast[l, r0:r0 + n, :]] * (SUB // LANES), axis=1) * tail[e:e + 1]
                if e >= N_REFLECT:
                    h = h + term
                else:
                    head = term if head is None else head + term
            row = lax.broadcasted_iota(i32, (8, SUB), 0)
            slots = jnp.concatenate([h[:8] + head, h[8:],
                                     jnp.where(row == 0, 1.0, tail[n_vpu - 1:n_vpu + 7]),
                                     tail[n_vpu + 7:]], axis=0).astype(bf16)
            if l == L - 2 and between is not None:
                between()
            g = jnp.dot(pltpu.bitcast(u_aug[:, l * LANES:(l + 1) * LANES], bf16), slots,
                        preferred_element_type=f32)

            x0 = x_buf[:, cols].astype(f32)
            x = x0 if l == 0 else pltpu.bitcast(state[...], bf16).astype(f32)
            x = (x0 * g + x).astype(bf16)
            if l < L - 1:
                state[...] = pltpu.bitcast(x, u32)

        for r0, r1, a, b in out_chunks:
            chunk = (pl.ds(r0, r1 - r0), columns(c0 + a, b - a))
            o_buf[chunk] = x[r0:r1, a:b]
            pltpu.make_async_copy(o_buf.at[chunk], o_hbm.at[chunk], o_sem).start()

    row_edges = (0, 32, 96, 224, D)
    early_chunks = [(r0, r1, 0, GROUP) for r0, r1 in zip(row_edges[:-1], row_edges[1:])] + [(0, D, GROUP, SUB)]

    def block(i, carry):
        first, second, rest = fetch(i)

        def between():
            rest.wait()

            @pl.when(i + 1 < n_blocks)
            def _():
                for copy in fetch(i + 1):
                    copy.start()

        n_sub = BLOCK // SUB
        for s in range(n_sub):
            cross_layers(i * BLOCK + s * SUB,
                         (first, second) if s == 0 else None,
                         between if s == 0 else None,
                         early_chunks if s == n_sub - 1 else [(0, D, 0, SUB)])
        return carry

    lax.fori_loop(0, n_blocks, block, 0)
    pltpu.make_async_copy(o_buf, o_hbm, o_sem).wait()


@jax.jit
def pallas_standalone__cross_network_dcn_v2__recsys_kernel(
    x0: jax.Array,
    U: jax.Array,
    V: jax.Array,
    bs: jax.Array,
):
    B, D = x0.shape
    L, _, R = U.shape
    KA = D // LANES * LANES
    n_vpu = D - KA - (LANES - R - 1)
    assert (D, R) == (416, 104) and B % BLOCK == 0 and L % 2 == 0 and 2 <= L <= 8
    assert all(a.dtype == bf16 for a in (x0, U, V, bs))

    out_t = pl.pallas_call(
        _kernel,
        in_specs=[pl.BlockSpec(memory_space=pltpu.HBM)] * 4,
        out_specs=pl.BlockSpec(memory_space=pltpu.HBM),
        out_shape=jax.ShapeDtypeStruct((D, B), bf16),
        scratch_shapes=[
            pltpu.VMEM((D, B + 2 * LANES), bf16),
            pltpu.VMEM((D, B), bf16),
            pltpu.VMEM((D // 2, SUB), u32),
            pltpu.VMEM((L, D, R), bf16),
            pltpu.VMEM((L, R, KA), bf16),
            pltpu.VMEM((L, R, D - KA), bf16),
            pltpu.VMEM((L, D), bf16),
            pltpu.VMEM((L, R, KA), f32),
            pltpu.VMEM((D // 2, L * LANES), u32),
            pltpu.VMEM((L, sum(_t_rows(n_vpu - 1, R)), LANES), f32),
            pltpu.VMEM((8 * 16, LANES), f32),
            pltpu.VMEM((8 * N_REFLECT, LANES), f32),
            pltpu.VMEM((8 * N_REFLECT, LANES), f32),
            pltpu.VMEM((8 * n_vpu, LANES), f32),
            pltpu.VMEM((L, R, LANES), f32),
            pltpu.VMEM((L, R, LANES), f32),
            pltpu.VMEM((8, LANES), f32),
            pltpu.SemaphoreType.DMA((3,)),
            pltpu.SemaphoreType.DMA(()),
            pltpu.SemaphoreType.DMA((3,)),
        ],
        compiler_params=pltpu.CompilerParams(
            vmem_limit_bytes=64 * 1024 * 1024,
            disable_bounds_checks=True,
            flags={"XLA_TPU_RESCHEDULE_DMA_DONES": True},
        ),
    )(x0.T, U, V, bs)
    return out_t.T
```
